```python
import os as _os
_os.environ.setdefault("JAX_PLATFORMS", "cpu")
import jax
import jax.numpy as jnp

def _softmax(x, axis=-1):
    return jax.nn.softmax(x, axis=axis)
def _gelu(x):
    return jax.nn.gelu(x, approximate=True)
def _silu(x):
    return jax.nn.silu(x)
def _sigmoid(x):
    return jax.nn.sigmoid(x)
def _layernorm(x, axis=-1, eps=1e-5):
    m = jnp.mean(x, axis=axis, keepdims=True)
    v = jnp.var(x, axis=axis, keepdims=True)
    return (x - m) / jnp.sqrt(v + eps)
def _scatter_add(tgt, idx, src, axis=0):
    return tgt.at[idx].add(src)
def _segment_sum(src, seg, n):
    return jax.ops.segment_sum(src, seg, n)
class _Rng:
    def __init__(self, key):
        self._k = key
    def _next(self):
        self._k, sub = jax.random.split(self._k)
        return sub
    def normal(self, shape):
        return jax.random.normal(self._next(), shape, dtype=jnp.bfloat16)
    def randint(self, lo, hi, shape):
        return jax.random.randint(self._next(), shape, lo, hi, dtype=jnp.int32)
    def uniform(self, shape, lo=0.0, hi=1.0):
        return jax.random.uniform(self._next(), shape, jnp.bfloat16, lo, hi)
    def permutation(self, n):
        return jax.random.permutation(self._next(), n)


kernel_name = 'sequential_preLN__linear_kernel_hedgehog__geglu_ffn__prompt'

def setup_inputs():
    _rng = _Rng(jax.random.key(int.from_bytes(__import__("os").urandom(4), "little")))
    _w = (lambda a: (lambda t: t.astype(jnp.bfloat16) if jnp.issubdtype(t.dtype, jnp.floating) else t)(jnp.asarray(a)))
    def _A_setup():
        B, S, D, H = 1, 2048, 640, 32
        Dh = D // H
        return {
            "x": _w((lambda *s: _rng.normal(s) * 0.05)(B, S, D)),
            "wqkv": _w((lambda *s: _rng.normal(s) * 0.2)(D, 3 * D)),
            "w_phi": _w((lambda *s: _rng.normal(s) * 0.2)(H, Dh, Dh) * (Dh ** -0.5)),
            "wo": _w((lambda *s: _rng.normal(s) * 0.05)(D, D)),
        }
    _A_in = _A_setup()

    def _B_setup():
        B, S, D, F = 1, 2048, 640, 1536
        return {
            "x": _w((lambda *s: _rng.normal(s) * 0.05)(B, S, D)),
            "w_gate": _w((lambda *s: _rng.normal(s) * 0.05)(D, F)),
            "w_up": _w((lambda *s: _rng.normal(s) * 0.05)(D, F)),
            "w_down": _w((lambda *s: _rng.normal(s) * 0.05)(F, D)),
        }
    _B_in = _B_setup()

    return {
        "A_x": _A_in["x"],
        "A_wqkv": _A_in["wqkv"],
        "A_w_phi": _A_in["w_phi"],
        "A_wo": _A_in["wo"],
        "B_x": _B_in["x"],
        "B_w_gate": _B_in["w_gate"],
        "B_w_up": _B_in["w_up"],
        "B_w_down": _B_in["w_down"],
    }

def reference(A_x, A_wqkv, A_w_phi, A_wo, B_x, B_w_gate, B_w_up, B_w_down):
    def _A_ref(x, wqkv, w_phi, wo):
        B, S, D = x.shape
        H = 32; Dh = D // H
        qkv = (lambda x, *d: x.transpose(*d))((x @ wqkv).reshape(B, S, 3, H, Dh), 2, 0, 3, 1, 4)
        q, k, v = qkv[0], qkv[1], qkv[2]
        pq = jnp.einsum("bhsd,hdf->bhsf", q, w_phi)
        pk = jnp.einsum("bhsd,hdf->bhsf", k, w_phi)
        phi_q = jnp.concatenate([_softmax(pq, axis=-1), _softmax(-pq, axis=-1)], axis=-1)
        phi_k = jnp.concatenate([_softmax(pk, axis=-1), _softmax(-pk, axis=-1)], axis=-1)
        kv = jnp.einsum("bhsf,bhsd->bhfd", phi_k, v)
        z  = jnp.einsum("bhsf->bhf", phi_k)
        num = jnp.einsum("bhqf,bhfd->bhqd", phi_q, kv)
        den = jnp.einsum("bhqf,bhf->bhq", phi_q, z)[..., None] + 1e-6
        o = num / den
        return (lambda x, *d: x.transpose(*d))(o, 0, 2, 1, 3).reshape(B, S, D) @ wo

    def _B_ref(x, w_gate, w_up, w_down):
        return (_gelu(x @ w_gate) * (x @ w_up)) @ w_down

    x = A_x
    h = x + _A_ref(_layernorm(x, axis=-1), A_wqkv, A_w_phi, A_wo)
    h2 = h + _B_ref(_layernorm(h, axis=-1), B_w_gate, B_w_up, B_w_down)
    return h2
```

```python
import functools

import jax
import jax.numpy as jnp
from jax import lax
import jax.experimental.pallas as pl
import jax.experimental.pallas.tpu as pltpu

_H = 32
_T = 512
_LN_ROWS = 64
_WO_ROWS = 128
_FFN_ROWS = 64
_LOG2E = 1.4426950408889634
_NT = (((1,), (1,)), ((), ()))
_F32 = jnp.float32
_BF16 = jnp.bfloat16


def _iota(shape, axis):
    return lax.broadcasted_iota(jnp.int32, shape, axis)


def _dot(a, b):
    return jnp.dot(a, b, preferred_element_type=_F32)


def _dot_nt(a, b):
    return lax.dot_general(a, b, _NT, preferred_element_type=_F32)


def _layernorm(x):
    m = jnp.mean(x, axis=-1, keepdims=True)
    c = x - m
    v = jnp.mean(c * c, axis=-1, keepdims=True)
    return c * lax.rsqrt(v + 1e-5)


def _head_allreduce(tiles, op):
    m = functools.reduce(op, tiles)
    m = op(m, pltpu.roll(m, 4, 0))
    return op(m, pltpu.roll(m, 2, 0))


def _dual_softmax(p):
    tiles = [p[j:j + 8, :] for j in range(0, p.shape[0], 8)]
    mx = _head_allreduce(tiles, jnp.maximum)
    mn = _head_allreduce(tiles, jnp.minimum)
    ep = [jnp.exp2(s - mx) for s in tiles]
    en = [jnp.exp2(mn - s) for s in tiles]
    rp = 1.0 / _head_allreduce(ep, jnp.add)
    rn = 1.0 / _head_allreduce(en, jnp.add)
    return jnp.concatenate([e * rp for e in ep] + [e * rn for e in en], axis=0)


def _gelu(x):
    c0 = 0.7978845608028654
    c1 = 0.7978845608028654 * 0.044715
    return (0.5 * x) * (1.0 + jnp.tanh(x * (c0 + c1 * (x * x))))


def _kernel(x_hbm, wqkv_hbm, wphi_hbm, wo_hbm, wg_hbm, wu_hbm, wd_hbm, out_hbm,
            x_v, wqkv_v, wphi_v, wo_v, wg_v, wu_v, wd_v, wt_v, stage_v, xn_v,
            phiq_v, phik_v, va_v, kv_v, h_v, hn_v, out_v, sem_x, sem_w, sem_o):
    S, D = x_v.shape
    T = _T
    dh = D // _H
    npair = _H // 2
    R = 2 * dh
    RA = R + 8
    nk = D // 128
    n = S // T
    Q, K, V = 0, 1, 2

    def x_copy(i):
        return pltpu.make_async_copy(x_hbm.at[pl.ds(i * T, T)], x_v.at[pl.ds(i * T, T)], sem_x.at[i])

    wqkv_copy = [pltpu.make_async_copy(wqkv_hbm.at[:, pl.ds(j * D, D)], wqkv_v.at[j], sem_w.at[j])
                 for j in range(3)]
    wphi_copy, wo_copy, *ffn_copies = [
        pltpu.make_async_copy(src, dst, sem_w.at[3 + j]) for j, (src, dst) in enumerate(
            [(wphi_hbm, wphi_v), (wo_hbm, wo_v), (wg_hbm, wg_v), (wu_hbm, wu_v), (wd_hbm, wd_v)])]

    def tokens(i):
        return pl.ds(pl.multiple_of(i * T, T), T)

    wphi_copy.start()
    x_copy(0).start()
    wqkv_copy[K].start()
    wphi_copy.wait()

    stage_v[...] = jnp.zeros(stage_v.shape, _F32)
    for d in range(dh):
        stage_v[pl.ds(0, dh), pl.ds(d * _H, _H)] = wphi_v[d].astype(_F32)
    r = _iota((D, D), 0)
    spread = (_iota((D, D), 1) == dh * (r % _H) + r // _H).astype(_BF16)
    wf = _dot(stage_v[...].astype(_BF16), spread)
    twice = (_iota((RA, 32), 0) // 2 == _iota((RA, 32), 1)).astype(_BF16)
    wf = _dot(twice, wf.astype(_BF16))[:R]
    off = _iota((R, 128), 1) - dh * (_iota((R, 128), 0) % 2)
    pairs_of = [range((128 * k) // R, (128 * k + 127) // R + 1) for k in range(nk)]
    maps = []
    for k in range(nk):
        blocks = []
        for p in pairs_of[k]:
            o = off + (128 * k - R * p)
            blocks.append(jnp.where((o >= 0) & (o < dh), wf[:, 128 * k:128 * k + 128], 0.0))
        maps.append(jnp.concatenate(blocks, axis=0).astype(_BF16))

    def fold(j):
        parts = [[] for _ in range(npair)]
        for k in range(nk):
            w = _dot_nt(maps[k], wqkv_v[j, :, pl.ds(128 * k, 128)])
            for m, p in enumerate(pairs_of[k]):
                parts[p].append(w[m * R:(m + 1) * R, :])
        for p in range(0, npair, 2):
            w = jnp.concatenate([functools.reduce(jnp.add, parts[p]),
                                 functools.reduce(jnp.add, parts[p + 1])], axis=0)
            wt_v[pl.ds(j * D + p * R, 2 * R), :] = (w * _LOG2E).astype(_BF16)

    def norm_x(i):
        for c in range(0, T, _LN_ROWS):
            x = x_v[pl.ds(pl.multiple_of(i * T + c, _LN_ROWS), _LN_ROWS), :]
            xn_v[i % 2, pl.ds(c, _LN_ROWS), :] = _layernorm(x.astype(_F32)).astype(_BF16)

    def project(j, i, p0, pairs):
        return _dot_nt(wt_v[pl.ds(j * D + p0 * R, pairs * R), :], xn_v[i % 2])

    def features(j, i, dst, pairs=npair):
        for p0 in range(0, npair, pairs):
            pr = project(j, i, p0, pairs)
            for p in range(pairs):
                dst[p0 + p, :, tokens(i)] = _dual_softmax(pr[p * R:(p + 1) * R, :]).astype(_BF16)

    def values(i):
        vt = project(V, i, 0, npair)
        ones = jnp.ones((8, T), _F32)
        for p in range(npair):
            va_v[p, :, tokens(i)] = jnp.concatenate([vt[p * R:(p + 1) * R, :], ones], axis=0).astype(_BF16)

    x_copy(0).wait()
    wqkv_copy[Q].start()
    norm_x(0)
    wqkv_copy[K].wait()
    wqkv_copy[V].start()
    x_copy(1).start()
    fold(K)
    features(K, 0, phik_v, pairs=2)
    wqkv_copy[Q].wait()
    wqkv_copy[V].wait()
    x_copy(1).wait()
    for i in range(2, n):
        x_copy(i).start()
    wo_copy.start()
    fold(Q)
    wt_v[pl.ds(V * D, D), :] = wqkv_v[V].T
    features(Q, 0, phiq_v, pairs=4)
    norm_x(1)
    values(0)
    for i in range(2, n):
        x_copy(i).wait()
    wo_copy.wait()
    for c in ffn_copies:
        c.start()

    def phase1(i):
        features(K, i, phik_v)
        features(Q, i, phiq_v)
        values(i)

    @pl.loop(1, n - 1)
    def _(i):
        phase1(i)
        norm_x(i + 1)

    phase1(n - 1)

    rr = _iota((RA, 2 * R), 0)
    second = ((rr >= dh) & (rr < R)) | (rr >= R + 4)
    same_head = second.astype(jnp.int32) == _iota((RA, 2 * R), 1) % 2
    for p in range(npair):
        kv_v[p] = jnp.where(same_head, _dot_nt(va_v[p], phik_v[p]), 0.0).astype(_BF16)

    for c in ffn_copies:
        c.wait()

    @pl.loop(0, n)
    def _(i):
        low = _iota((8, T), 0) < 4
        outs = []
        for p in range(npair):
            nd = _dot(kv_v[p], phiq_v[p, :, tokens(i)])
            r01 = 1.0 / (nd[R:RA, :] + 1e-6)
            r10 = pltpu.roll(r01, 4, 0)
            r0 = jnp.where(low, r01, r10)
            r1 = jnp.where(low, r10, r01)
            outs += [nd[8 * j:8 * j + 8, :] * s for j, s in enumerate((r0, r0, r01, r1, r1))]
        o = jnp.concatenate(outs, axis=0).T.astype(_BF16)
        a = jnp.concatenate([_dot(o[c:c + _WO_ROWS, :], wo_v[...]) for c in range(0, T, _WO_ROWS)], axis=0)
        for c in range(0, T, _LN_ROWS):
            x = x_v[pl.ds(pl.multiple_of(i * T + c, _LN_ROWS), _LN_ROWS), :]
            h = x.astype(_F32) + a[c:c + _LN_ROWS, :]
            h_v[pl.ds(c, _LN_ROWS), :] = h
            hn_v[pl.ds(c, _LN_ROWS), :] = _layernorm(h).astype(_BF16)
        for c in range(0, T, _FFN_ROWS):
            hn = hn_v[pl.ds(c, _FFN_ROWS), :]
            act = (_gelu(_dot(hn, wg_v[...])) * _dot(hn, wu_v[...])).astype(_BF16)
            y = h_v[pl.ds(c, _FFN_ROWS), :] + _dot(act, wd_v[...])
            rows = pl.ds(pl.multiple_of(i * T + c, _FFN_ROWS), _FFN_ROWS)
            out_v[rows, :] = y.astype(out_v.dtype)
            pltpu.make_async_copy(out_v.at[rows], out_hbm.at[rows], sem_o.at[0]).start()

    pltpu.make_async_copy(out_v, out_hbm, sem_o.at[0]).wait()


@jax.jit
def pallas_sequential_preLN__linear_kernel_hedgehog__geglu_ffn__prompt_kernel(
    A_x: jax.Array,
    A_wqkv: jax.Array,
    A_w_phi: jax.Array,
    A_wo: jax.Array,
    B_x: jax.Array,
    B_w_gate: jax.Array,
    B_w_up: jax.Array,
    B_w_down: jax.Array,
):
    del B_x
    B, S, D = A_x.shape
    F = B_w_gate.shape[1]
    dh = D // _H
    npair = _H // 2
    R = 2 * dh
    assert B == 1 and dh == 20 and S % _T == 0 and S // _T >= 3
    hbm = pl.BlockSpec(memory_space=pl.ANY)
    out = pl.pallas_call(
        _kernel,
        out_shape=jax.ShapeDtypeStruct((S, D), A_x.dtype),
        in_specs=[hbm] * 7,
        out_specs=hbm,
        scratch_shapes=[
            pltpu.VMEM((S, D), _BF16),
            pltpu.VMEM((3, D, D), _BF16),
            pltpu.VMEM((dh, dh, _H), _BF16),
            pltpu.VMEM((D, D), _BF16),
            pltpu.VMEM((D, F), _BF16),
            pltpu.VMEM((D, F), _BF16),
            pltpu.VMEM((F, D), _BF16),
            pltpu.VMEM((3 * D, D), _BF16),
            pltpu.VMEM((32, D), _F32),
            pltpu.VMEM((2, _T, D), _BF16),
            pltpu.VMEM((npair, 2 * R, S), _BF16),
            pltpu.VMEM((npair, 2 * R, S), _BF16),
            pltpu.VMEM((npair, R + 8, S), _BF16),
            pltpu.VMEM((npair, R + 8, 2 * R), _BF16),
            pltpu.VMEM((_T, D), _F32),
            pltpu.VMEM((_T, D), _BF16),
            pltpu.VMEM((S, D), A_x.dtype),
            pltpu.SemaphoreType.DMA((S // _T,)),
            pltpu.SemaphoreType.DMA((8,)),
            pltpu.SemaphoreType.DMA((1,)),
        ],
        compiler_params=pltpu.CompilerParams(vmem_limit_bytes=100 * 1024 * 1024),
    )(A_x.reshape(S, D), A_wqkv, A_w_phi.transpose(1, 2, 0), A_wo, B_w_gate, B_w_up, B_w_down)
    return out.reshape(B, S, D)
```
